```python
import jax
import jax.numpy as jnp

def _softmax(x, axis=-1):
    return jax.nn.softmax(x, axis=axis)
def _gelu(x):
    return jax.nn.gelu(x, approximate=True)
def _silu(x):
    return jax.nn.silu(x)
def _sigmoid(x):
    return jax.nn.sigmoid(x)
def _layernorm(x, axis=-1, eps=1e-5):
    m = jnp.mean(x, axis=axis, keepdims=True)
    v = jnp.var(x, axis=axis, keepdims=True)
    return (x - m) / jnp.sqrt(v + eps)
def _scatter_add(tgt, idx, src, axis=0):
    return tgt.at[idx].add(src)
def _segment_sum(src, seg, n):
    return jax.ops.segment_sum(src, seg, n)
class _Rng:
    def __init__(self, key):
        self._k = key
    def _next(self):
        self._k, sub = jax.random.split(self._k)
        return sub
    def normal(self, shape):
        return jax.random.normal(self._next(), shape, dtype=jnp.bfloat16)
    def randint(self, lo, hi, shape):
        return jax.random.randint(self._next(), shape, lo, hi, dtype=jnp.int32)
    def uniform(self, shape, lo=0.0, hi=1.0):
        return jax.random.uniform(self._next(), shape, jnp.bfloat16, lo, hi)
    def permutation(self, n):
        return jax.random.permutation(self._next(), n)


kernel_name = 'recurrent_scan__sliding_block_cached__mixer_s_mlp__decode'

def setup_inputs():
    _rng = _Rng(jax.random.key(int.from_bytes(__import__("os").urandom(4), "little")))
    _w = (lambda a: (lambda t: t.astype(jnp.bfloat16) if jnp.issubdtype(t.dtype, jnp.floating) else t)(jnp.asarray(a)))
    def _A_setup():
        B, Sq, D = 1, 1, 512
        Hq, Hkv, Sk, Dh = 32, 32, 32768, 128
        assert Hq % Hkv == 0, (Hq, Hkv)
        return {
            "x": _w((lambda *s: _rng.normal(s) * 0.05)(B, Sq, D)),
            "k_cache": _w((lambda *s: _rng.normal(s) * 0.05)(B, Hkv, Sk, Dh)),
            "v_cache": _w((lambda *s: _rng.normal(s) * 0.05)(B, Hkv, Sk, Dh)),
            "wq": _w((lambda *s: _rng.normal(s) * 0.05)(D, Hq * Dh) * (D ** -0.5)),
            "wo": _w((lambda *s: _rng.normal(s) * 0.05)(Hq * Dh, D) * ((Hq * Dh) ** -0.5)),
        }
    _A_in = _A_setup()

    def _B_setup():
        B, S, D, F = 1, 1, 512, 1376
        return {
            "x":  _w((lambda *s: _rng.normal(s) * 0.05)(B, S, D)),
            "w1": _w((lambda *s: _rng.normal(s) * 0.05)(D, D) * (D ** -0.5)),
            "w2": _w((lambda *s: _rng.normal(s) * 0.05)(D, D) * (D ** -0.5)),
            "w3": _w((lambda *s: _rng.normal(s) * 0.05)(D, F) * (D ** -0.5)),
            "w4": _w((lambda *s: _rng.normal(s) * 0.05)(F, D) * (F ** -0.5)),
        }
    _B_in = _B_setup()

    return {
        "A_x": _A_in["x"],
        "A_k_cache": _A_in["k_cache"],
        "A_v_cache": _A_in["v_cache"],
        "A_wq": _A_in["wq"],
        "A_wo": _A_in["wo"],
        "B_x": _B_in["x"],
        "B_w1": _B_in["w1"],
        "B_w2": _B_in["w2"],
        "B_w3": _B_in["w3"],
        "B_w4": _B_in["w4"],
    }

def reference(A_x, A_k_cache, A_v_cache, A_wq, A_wo, B_x, B_w1, B_w2, B_w3, B_w4):
    def _A_ref(x, k_cache, v_cache, wq, wo):
        B, Sq, D = x.shape
        Hq, Dh = 32, 128
        Hkv, Sk = k_cache.shape[1], k_cache.shape[2]
        W = min(4096, max(256, Sk // 4))
        rep = Hq // Hkv
        q = (lambda x, *d: x.transpose(*d))((x @ wq).reshape(B, Sq, Hq, Dh), 0, 2, 1, 3)
        k = jnp.repeat(k_cache[:, :, Sk - W:, :], rep, axis=1)
        v = jnp.repeat(v_cache[:, :, Sk - W:, :], rep, axis=1)
        scores = jnp.einsum("bhqd,bhkd->bhqk", q, k) * (Dh ** -0.5)
        p = _softmax(scores, axis=-1)
        o = jnp.einsum("bhqk,bhkd->bhqd", p, v)
        return (lambda x, *d: x.transpose(*d))(o, 0, 2, 1, 3).reshape(B, Sq, Hq * Dh) @ wo

    def _B_ref(x, w1, w2, w3, w4):
        B, S, D = x.shape
        h = _gelu(_layernorm(x, axis=-1) @ w1)
        c = D // 4
        g0 = jnp.pad(h[:, :, 0*c:1*c], ((0, 0), (1, 0), (0, 0)))[:, :S, :]
        g1 = jnp.pad(h[:, :, 1*c:2*c], ((0, 0), (0, 1), (0, 0)))[:, 1:, :]
        g2 = jnp.pad(h[:, :, 2*c:3*c], ((0, 0), (2, 0), (0, 0)))[:, :S, :]
        g3 = jnp.pad(h[:, :, 3*c:   ], ((0, 0), (0, 2), (0, 0)))[:, 2:, :]
        hs = jnp.concatenate([g0, g1, g2, g3], axis=-1) @ w2
        x1 = x + hs
        h2 = _gelu(_layernorm(x1, axis=-1) @ w3) @ w4
        return x1 + h2

    x = A_x
    xn = _layernorm(x, axis=-1)
    s = _A_ref(xn, A_k_cache, A_v_cache, A_wq, A_wo)
    g = _silu(_B_ref(xn, B_w1, B_w2, B_w3, B_w4))
    return x + s * g
```

```python
import jax
import jax.numpy as jnp
from jax import lax
import jax.experimental.pallas as pl
import jax.experimental.pallas.tpu as pltpu

_EPS = 1e-5
_KV_ROWS = 128
_AHEAD = 16
_WO_HEADS = 2
_PRE_WQ = 40
_NSLOT = 3


def _layernorm(x):
    m = jnp.mean(x, axis=-1, keepdims=True)
    d = x - m
    v = jnp.mean(d * d, axis=-1, keepdims=True)
    return d / jnp.sqrt(v + _EPS)


@jax.jit
def pallas_recurrent_scan__sliding_block_cached__mixer_s_mlp__decode_kernel(
    A_x: jax.Array,
    A_k_cache: jax.Array,
    A_v_cache: jax.Array,
    A_wq: jax.Array,
    A_wo: jax.Array,
    B_x: jax.Array,
    B_w1: jax.Array,
    B_w2: jax.Array,
    B_w3: jax.Array,
    B_w4: jax.Array,
):
    B, Sq, D = A_x.shape
    _, H, Sk, Dh = A_k_cache.shape
    assert B == 1 and Sq == 1
    W = min(4096, max(256, Sk // 4))
    F = B_w3.shape[1]
    HD = H * Dh
    scale = Dh ** -0.5
    bf16 = jnp.bfloat16
    f32 = jnp.float32

    nch = W // _KV_ROWS
    chunk_bytes = _KV_ROWS * Dh * 2
    wrows = chunk_bytes // (D * 2)
    wq_cols = HD // 2
    wq_rows = chunk_bytes // (wq_cols * 2)
    assert F % wrows == 0 and HD % (2 * wrows) == 0
    assert wq_rows % 8 == 0 and D % wq_rows == 0
    n_wq = D // wq_rows
    n_wo = HD // (2 * wrows)
    wo_group_rows = _WO_HEADS * Dh
    wo_pairs_per_group = wo_group_rows // (2 * wrows)
    n_wo_groups = H // _WO_HEADS
    assert n_wo == 2 * nch and _PRE_WQ <= n_wq

    def kernel(x_hbm, k_hbm, v_hbm, wq_hbm, wo_hbm, w3t_hbm, w4_hbm, o_ref,
               xbuf, kbuf, vbuf, wqbuf, wobuf, w3buf, w4buf, q_scr, o_scr,
               sem_x, sem_w, sem_kv, sem_wo):

        def wait_all(buf, sem):
            pltpu.make_async_copy(buf, buf, sem).wait()

        def loop(lo, hi, f):
            def body(i, c):
                f(i)
                return c
            lax.fori_loop(lo, hi, body, 0)

        def kv_pair(h, slot, c):
            st = c * _KV_ROWS
            if not isinstance(c, int):
                st = pl.multiple_of(st, _KV_ROWS)
            pltpu.make_async_copy(
                k_hbm.at[0, h, pl.ds(Sk - W + st, _KV_ROWS), :],
                kbuf.at[slot, pl.ds(st, _KV_ROWS), :],
                sem_kv.at[0, slot]).start(priority=0)
            pltpu.make_async_copy(
                v_hbm.at[0, h, pl.ds(Sk - W + st, _KV_ROWS), :],
                vbuf.at[slot, pl.ds(st, _KV_ROWS), :],
                sem_kv.at[1, slot]).start(priority=1)

        def mlp_pair(c):
            r = pl.multiple_of(c * wrows, wrows)
            pltpu.make_async_copy(w3t_hbm.at[pl.ds(r, wrows), :],
                                  w3buf.at[pl.ds(r, wrows), :],
                                  sem_w.at[0]).start(priority=0)
            pltpu.make_async_copy(w4_hbm.at[pl.ds(r, wrows), :],
                                  w4buf.at[pl.ds(r, wrows), :],
                                  sem_w.at[1]).start(priority=1)

        def wq_pair(j):
            r = pl.multiple_of(j * wq_rows, wq_rows)
            for p in range(2):
                pltpu.make_async_copy(
                    wq_hbm.at[pl.ds(r, wq_rows), pl.ds(p * wq_cols, wq_cols)],
                    wqbuf.at[pl.ds(r, wq_rows), pl.ds(p * wq_cols, wq_cols)],
                    sem_w.at[2]).start(priority=p)

        def wo_pair(j):
            for p in range(2):
                r = pl.multiple_of((2 * j + p) * wrows, wrows)
                pltpu.make_async_copy(wo_hbm.at[pl.ds(r, wrows), :],
                                      wobuf.at[pl.ds(r, wrows), :],
                                      sem_wo.at[j // wo_pairs_per_group]).start(priority=p)

        x_copy = pltpu.make_async_copy(x_hbm, xbuf, sem_x.at[0])
        x_copy.start()
        loop(0, F // wrows, mlp_pair)
        x_copy.wait()
        x = xbuf[0].astype(f32)
        xn = _layernorm(x)
        x1n = _layernorm(xn)
        loop(0, _PRE_WQ, wq_pair)
        wait_all(w3buf, sem_w.at[0])
        wait_all(w4buf, sem_w.at[1])
        hh = lax.dot_general(x1n.astype(bf16), w3buf[...], (((1,), (1,)), ((), ())),
                             preferred_element_type=f32)
        hh = jax.nn.gelu(hh, approximate=True)
        h2 = jnp.dot(hh.astype(bf16), w4buf[...], preferred_element_type=f32)
        gate = jax.nn.silu(xn + h2)

        loop(_PRE_WQ, n_wq, wq_pair)
        loop(0, nch, lambda c: kv_pair(0, 0, c))
        wait_all(wqbuf, sem_w.at[2])
        loop(0, _AHEAD, lambda c: kv_pair(1, 1, c))
        q = jnp.dot(xn.astype(bf16), wqbuf[...], preferred_element_type=f32).astype(bf16)
        for h in range(H):
            q_scr[h] = q[:, h * Dh:(h + 1) * Dh]

        def head(h, carry):
            slot = lax.rem(h, _NSLOT)
            slot1 = lax.rem(h + 1, _NSLOT)
            slot2 = lax.rem(h + 2, _NSLOT)

            wait_all(kbuf.at[slot], sem_kv.at[0, slot])

            @pl.when(h + 1 < H)
            def _():
                for c in range(_AHEAD, nch):
                    kv_pair(h + 1, slot1, c)

            @pl.when(h + 2 < H)
            def _():
                for c in range(_AHEAD):
                    kv_pair(h + 2, slot2, c)

            wlo = jnp.where(h == H - 2, 0, _AHEAD)
            whi = jnp.where(h == H - 2, _AHEAD,
                            jnp.where(h == H - 1, nch + _AHEAD, _AHEAD))
            loop(wlo, whi, wo_pair)

            s = lax.dot_general(q_scr[h], kbuf[slot], (((1,), (1,)), ((), ())),
                                preferred_element_type=f32) * scale
            m = jnp.max(s, axis=-1, keepdims=True)
            p = jnp.exp(s - m)
            l = jnp.sum(p, axis=-1, keepdims=True)
            wait_all(vbuf.at[slot], sem_kv.at[1, slot])
            o = jnp.dot(p.astype(bf16), vbuf[slot], preferred_element_type=f32)
            o_scr[h] = (o / l).astype(bf16)
            return carry

        lax.fori_loop(0, H, head, 0)
        loop(nch + _AHEAD, n_wo, wo_pair)

        def wo_group(gi, acc):
            r0 = pl.multiple_of(gi * wo_group_rows, wo_group_rows)
            wg = wobuf.at[pl.ds(r0, wo_group_rows), :]
            wait_all(wg, sem_wo.at[gi])
            og = jnp.concatenate(
                [o_scr[gi * _WO_HEADS + t] for t in range(_WO_HEADS)], axis=1)
            return acc + jnp.dot(og, wg[...], preferred_element_type=f32)

        s_out = lax.fori_loop(0, n_wo_groups, wo_group, jnp.zeros((1, D), f32))
        o_ref[0] = (x + s_out * gate).astype(o_ref.dtype)

    return pl.pallas_call(
        kernel,
        in_specs=[pl.BlockSpec(memory_space=pl.ANY)] * 7,
        out_specs=pl.BlockSpec(memory_space=pltpu.VMEM),
        out_shape=jax.ShapeDtypeStruct((B, Sq, D), A_x.dtype),
        scratch_shapes=[
            pltpu.VMEM((1, 1, D), bf16),
            pltpu.VMEM((_NSLOT, W, Dh), bf16),
            pltpu.VMEM((_NSLOT, W, Dh), bf16),
            pltpu.VMEM((D, HD), bf16),
            pltpu.VMEM((HD, D), bf16),
            pltpu.VMEM((F, D), bf16),
            pltpu.VMEM((F, D), bf16),
            pltpu.VMEM((H, 1, Dh), bf16),
            pltpu.VMEM((H, 1, Dh), bf16),
            pltpu.SemaphoreType.DMA((1,)),
            pltpu.SemaphoreType.DMA((3,)),
            pltpu.SemaphoreType.DMA((2, _NSLOT)),
            pltpu.SemaphoreType.DMA((n_wo_groups,)),
        ],
        compiler_params=pltpu.CompilerParams(
            vmem_limit_bytes=64 * 1024 * 1024,
            disable_bounds_checks=True,
            disable_semaphore_checks=True,
        ),
    )(A_x, A_k_cache, A_v_cache, A_wq, A_wo, B_w3.T, B_w4)
```

```python
import functools, contextlib
import jax
import jax.numpy as jnp
from jax import lax
import jax.experimental.pallas as pl
import jax.experimental.pallas.tpu as pltpu

_EPS = 1e-5


def _layernorm(x):
    m = jnp.mean(x, axis=-1, keepdims=True)
    d = x - m
    v = jnp.mean(d * d, axis=-1, keepdims=True)
    return d / jnp.sqrt(v + _EPS)


def build(G=8, KV_ROWS=128, AHEAD=64, WO_HEADS=2, PRE_WQ=40, scopes=False, skip_compute=False,
          TAIL=(4, 12), MS=True, PRE_R=10):
    def fn(A_x, A_k_cache, A_v_cache, A_wq, A_wo, B_x, B_w1, B_w2, B_w3, B_w4):
        B, Sq, D = A_x.shape
        _, H, Sk, Dh = A_k_cache.shape
        W = min(4096, max(256, Sk // 4))
        F = B_w3.shape[1]
        HD = H * Dh
        scale = Dh ** -0.5
        bf16 = jnp.bfloat16
        f32 = jnp.float32
        NG = H // G
        nblk = W // KV_ROWS
        RPT = nblk // G
        AR = AHEAD // G
        assert nblk % G == 0 and AHEAD % G == 0 and AR % RPT == 0
        CB = KV_ROWS * Dh * 2
        wrows = CB // (D * 2)
        assert F % wrows == 0 and HD % (2 * wrows) == 0
        wq_cols = HD // 2
        wq_rows = CB // (wq_cols * 2)
        assert wq_rows % 8 == 0 and D % wq_rows == 0
        n_wq = D // wq_rows
        n_wo = HD // (2 * wrows)
        wo_pairs_per_group = (WO_HEADS * Dh) // (2 * wrows)
        n_wo_groups = H // WO_HEADS
        ppr = G // 2
        sc = jax.named_scope if scopes else (lambda n: contextlib.nullcontext())

        def kernel(x_hbm, k_hbm, v_hbm, wq_hbm, wo_hbm, w3t_hbm, w4_hbm, o_ref,
                   xbuf, kbuf, vbuf, wqbuf, wobuf, w3buf, w4buf, q_scr, p_scr, l_scr, o_scr,
                   sem_x, sem_w, sem_kv, sem_wo):

            def wait_all(buf, sem):
                pltpu.make_async_copy(buf, buf, sem).wait()

            def loop(lo, hi, f):
                def b(i, c):
                    f(i)
                    return c
                lax.fori_loop(lo, hi, b, 0)

            def kv_round(which, g, blk):
                src = (k_hbm, v_hbm)[which]
                dst = (kbuf, vbuf)[which]
                st = pl.multiple_of(blk * KV_ROWS, KV_ROWS)
                for j in range(G):
                    h = g * G + j
                    pltpu.make_async_copy(
                        src.at[0, h, pl.ds(Sk - W + st, KV_ROWS), :],
                        dst.at[h, pl.ds(st, KV_ROWS), :],
                        sem_kv.at[which, h]).start(priority=j % 2)

            def mlp_pair(c):
                r = pl.multiple_of(c * wrows, wrows)
                pltpu.make_async_copy(w3t_hbm.at[pl.ds(r, wrows), :], w3buf.at[pl.ds(r, wrows), :],
                                      sem_w.at[0]).start(priority=0)
                pltpu.make_async_copy(w4_hbm.at[pl.ds(r, wrows), :], w4buf.at[pl.ds(r, wrows), :],
                                      sem_w.at[1]).start(priority=1)

            def wq_pair(j):
                r = pl.multiple_of(j * wq_rows, wq_rows)
                for p in range(2):
                    pltpu.make_async_copy(
                        wq_hbm.at[pl.ds(r, wq_rows), pl.ds(p * wq_cols, wq_cols)],
                        wqbuf.at[pl.ds(r, wq_rows), pl.ds(p * wq_cols, wq_cols)],
                        sem_w.at[2]).start(priority=p)

            def wo_pair(j):
                for p in range(2):
                    r = pl.multiple_of((2 * j + p) * wrows, wrows)
                    pltpu.make_async_copy(wo_hbm.at[pl.ds(r, wrows), :], wobuf.at[pl.ds(r, wrows), :],
                                          sem_wo.at[j // wo_pairs_per_group]).start(priority=p)

            n_mlp = F // wrows
            MS_PER = -(-n_mlp // 4)

            def mlp_round(r):
                for s_ in range(4):
                    c = s_ * MS_PER + r
                    def go(c=c):
                        row = pl.multiple_of(c * wrows, wrows)
                        pltpu.make_async_copy(w3t_hbm.at[pl.ds(row, wrows), :], w3buf.at[pl.ds(row, wrows), :],
                                              sem_w.at[0]).start(priority=0)
                        pltpu.make_async_copy(w4_hbm.at[pl.ds(row, wrows), :], w4buf.at[pl.ds(row, wrows), :],
                                              sem_w.at[1]).start(priority=1)
                    if (s_ + 1) * MS_PER <= n_mlp:
                        go()
                    else:
                        pl.when(c < n_mlp)(go)

            def wq_round(i):
                col = pl.multiple_of((i % 2) * wq_cols, wq_cols)
                for s_ in range(8):
                    r = pl.multiple_of((s_ * (n_wq // 8) + i // 2) * wq_rows, wq_rows)
                    pltpu.make_async_copy(
                        wq_hbm.at[pl.ds(r, wq_rows), pl.ds(col, wq_cols)],
                        wqbuf.at[pl.ds(r, wq_rows), pl.ds(col, wq_cols)],
                        sem_w.at[2]).start(priority=s_ % 2)

            with sc("p_issue0"):
                pltpu.make_async_copy(x_hbm, xbuf, sem_x.at[0]).start()
                if MS:
                    loop(0, MS_PER, mlp_round)
                else:
                    loop(0, F // wrows, mlp_pair)
            with sc("p_ln"):
                pltpu.make_async_copy(x_hbm, xbuf, sem_x.at[0]).wait()
                x = xbuf[0].astype(f32)
                xn = _layernorm(x)
                x1n = _layernorm(xn)
            with sc("p_issue1"):
                if MS:
                    loop(0, PRE_R, wq_round)
                else:
                    loop(0, PRE_WQ, wq_pair)
            with sc("p_mlp"):
                wait_all(w3buf, sem_w.at[0])
                wait_all(w4buf, sem_w.at[1])
                if skip_compute:
                    g_ = x1n
                else:
                    hh = lax.dot_general(x1n.astype(bf16), w3buf[...], (((1,), (1,)), ((), ())),
                                         preferred_element_type=f32)
                    hh = jax.nn.gelu(hh, approximate=True)
                    h2 = jnp.dot(hh.astype(bf16), w4buf[...], preferred_element_type=f32)
                    g_ = jax.nn.silu(xn + h2)
            with sc("p_issue2"):
                if MS:
                    loop(PRE_R, 2 * n_wq // 8, wq_round)
                else:
                    loop(PRE_WQ, n_wq, wq_pair)
                loop(0, AR, lambda r: kv_round(0, 0, r))
            with sc("p_wqwait"):
                wait_all(wqbuf, sem_w.at[2])
            with sc("p_issue3"):
                loop(AR, AR + RPT, lambda r: kv_round(0, 0, r))
            with sc("p_q"):
                if not skip_compute:
                    q = jnp.dot(xn.astype(bf16), wqbuf[...], preferred_element_type=f32).astype(bf16)
                    for h in range(H):
                        q_scr[h] = q[:, h * Dh:(h + 1) * Dh]
            with sc("p_issue4"):
                loop(AR + RPT, nblk, lambda r: kv_round(0, 0, r))
                loop(0, AR, lambda r: kv_round(1, 0, r))

            NT = G - AR // RPT

            def group(g, carry):
                def ktask(j, c):
                    h = g * G + j
                    with sc("k_wait"):
                        wait_all(kbuf.at[h], sem_kv.at[0, h])
                    with sc("k_issue"):
                        @pl.when(j < NT)
                        def _():
                            loop(AR + RPT * j, AR + RPT * (j + 1), lambda r: kv_round(1, g, r))

                        @pl.when(jnp.logical_and(j >= NT, g < NG - 1))
                        def _():
                            loop(RPT * (j - NT), RPT * (j - NT + 1), lambda r: kv_round(0, g + 1, r))

                        @pl.when(jnp.logical_and(j >= NT, g == NG - 1))
                        def _():
                            loop(ppr * RPT * (j - NT), ppr * RPT * (j - NT + 1), wo_pair)
                    with sc("k_task"):
                        if not skip_compute:
                            s = lax.dot_general(q_scr[h], kbuf[h], (((1,), (1,)), ((), ())),
                                                preferred_element_type=f32) * scale
                            m = jnp.max(s, axis=-1, keepdims=True)
                            p = jnp.exp(s - m)
                            l_scr[j] = jnp.broadcast_to(jnp.sum(p, axis=-1, keepdims=True), (1, Dh))
                            p_scr[j] = p.astype(bf16)
                    return c

                lax.fori_loop(0, G, ktask, 0)

                def vtask(j, c):
                    h = g * G + j
                    with sc("v_wait"):
                        wait_all(vbuf.at[h], sem_kv.at[1, h])
                    with sc("v_issue"):
                        @pl.when(jnp.logical_and(j < NT, g < NG - 1))
                        def _():
                            loop(AR + RPT * j, AR + RPT * (j + 1), lambda r: kv_round(0, g + 1, r))

                        @pl.when(jnp.logical_and(j >= NT, g < NG - 1))
                        def _():
                            loop(RPT * (j - NT), RPT * (j - NT + 1), lambda r: kv_round(1, g + 1, r))

                        base = ppr * AR
                        lo = jnp.where(j == G // 2, base, base + TAIL[0] * 3)
                        hi = jnp.where(j == G // 2, base + TAIL[0] * 3, base + TAIL[0] * 3)
                        @pl.when(g == NG - 1)
                        def _():
                            loop(lo, hi, wo_pair)
                    with sc("v_task"):
                        if not skip_compute:
                            o = jnp.dot(p_scr[j], vbuf[h], preferred_element_type=f32)
                            o_scr[h] = (o / l_scr[j]).astype(bf16)
                    return c

                lax.fori_loop(0, G, vtask, 0)
                return carry

            lax.fori_loop(0, NG, group, 0)

            with sc("t_issue"):
                loop(ppr * AR + TAIL[0] * 3, n_wo, wo_pair)

            def wo_body(gi, acc):
                r0 = pl.multiple_of(gi * (WO_HEADS * Dh), WO_HEADS * Dh)
                wg = wobuf.at[pl.ds(r0, WO_HEADS * Dh), :]
                wait_all(wg, sem_wo.at[gi])
                if skip_compute:
                    return acc
                if WO_HEADS == 1:
                    og = o_scr[gi]
                else:
                    og = jnp.concatenate([o_scr[gi * WO_HEADS + t] for t in range(WO_HEADS)], axis=1)
                return acc + jnp.dot(og, wg[...], preferred_element_type=f32)

            with sc("t_wo"):
                acc = lax.fori_loop(0, n_wo_groups, wo_body, jnp.zeros((1, D), f32))
            with sc("t_final"):
                o_ref[0] = (x + acc * g_).astype(o_ref.dtype)

        return pl.pallas_call(
            kernel,
            in_specs=[pl.BlockSpec(memory_space=pl.ANY)] * 7,
            out_specs=pl.BlockSpec(memory_space=pltpu.VMEM),
            out_shape=jax.ShapeDtypeStruct((B, Sq, D), A_x.dtype),
            scratch_shapes=[
                pltpu.VMEM((1, 1, D), bf16),
                pltpu.VMEM((H, W, Dh), bf16),
                pltpu.VMEM((H, W, Dh), bf16),
                pltpu.VMEM((D, HD), bf16),
                pltpu.VMEM((HD, D), bf16),
                pltpu.VMEM((F, D), bf16),
                pltpu.VMEM((F, D), bf16),
                pltpu.VMEM((H, 1, Dh), bf16),
                pltpu.VMEM((G, 1, W), bf16),
                pltpu.VMEM((G, 1, Dh), f32),
                pltpu.VMEM((H, 1, Dh), bf16),
                pltpu.SemaphoreType.DMA((2,)),
                pltpu.SemaphoreType.DMA((3,)),
                pltpu.SemaphoreType.DMA((2, H)),
                pltpu.SemaphoreType.DMA((n_wo_groups,)),
            ],
            compiler_params=pltpu.CompilerParams(vmem_limit_bytes=100 * 1024 * 1024,
                                                 disable_bounds_checks=True,
                                                 disable_semaphore_checks=True),
        )(A_x, A_k_cache, A_v_cache, A_wq, A_wo, B_w3.T, B_w4)
    return fn


_fn = build(**dict())

@jax.jit
def pallas_recurrent_scan__sliding_block_cached__mixer_s_mlp__decode_kernel(A_x, A_k_cache, A_v_cache, A_wq, A_wo, B_x, B_w1, B_w2, B_w3, B_w4):
    return _fn(A_x, A_k_cache, A_v_cache, A_wq, A_wo, B_x, B_w1, B_w2, B_w3, B_w4)
```

```python
import functools, contextlib
import jax
import jax.numpy as jnp
from jax import lax
import jax.experimental.pallas as pl
import jax.experimental.pallas.tpu as pltpu

_EPS = 1e-5


def _layernorm(x):
    m = jnp.mean(x, axis=-1, keepdims=True)
    d = x - m
    v = jnp.mean(d * d, axis=-1, keepdims=True)
    return d / jnp.sqrt(v + _EPS)


def build(G=8, KV_ROWS=128, AHEAD=64, WO_HEADS=2, scopes=False, skip_compute=False,
          T0=12, T1=(4, 10), K0_SPLIT=16):
    def fn(A_x, A_k_cache, A_v_cache, A_wq, A_wo, B_x, B_w1, B_w2, B_w3, B_w4):
        B, Sq, D = A_x.shape
        _, H, Sk, Dh = A_k_cache.shape
        W = min(4096, max(256, Sk // 4))
        F = B_w3.shape[1]
        HD = H * Dh
        scale = Dh ** -0.5
        bf16 = jnp.bfloat16
        f32 = jnp.float32
        NG = H // G
        nblk = W // KV_ROWS
        RPT = nblk // G
        AR = AHEAD // G
        assert nblk % G == 0 and AHEAD % G == 0 and AR % RPT == 0
        CB = KV_ROWS * Dh * 2
        wrows = CB // (D * 2)
        assert F % wrows == 0 and HD % (2 * wrows) == 0
        wq_cols = HD // 2
        wq_rows = CB // (wq_cols * 2)
        assert wq_rows % 8 == 0 and D % wq_rows == 0
        n_wq = D // wq_rows
        n_wo = HD // (2 * wrows)
        wo_pairs_per_group = (WO_HEADS * Dh) // (2 * wrows)
        n_wo_groups = H // WO_HEADS
        ppr = G // 2
        n_mlp = F // wrows
        MS_PER = -(-n_mlp // 4)
        sc = jax.named_scope if scopes else (lambda n: contextlib.nullcontext())

        def kernel(x_hbm, k_hbm, v_hbm, wq_hbm, wo_hbm, w3t_hbm, w4_hbm, o_ref,
                   xbuf, kbuf, vbuf, wqbuf, wobuf, w3buf, w4buf, q_scr, p_scr, l_scr, o_scr,
                   sem_x, sem_w, sem_kv, sem_wo):

            def wait_all(buf, sem):
                pltpu.make_async_copy(buf, buf, sem).wait()

            def loop(lo, hi, f):
                def b(i, c):
                    f(i)
                    return c
                lax.fori_loop(lo, hi, b, 0)

            def kv_round(which, g, blk):
                src = (k_hbm, v_hbm)[which]
                dst = (kbuf, vbuf)[which]
                st = pl.multiple_of(blk * KV_ROWS, KV_ROWS)
                for j in range(G):
                    h = g * G + j
                    pltpu.make_async_copy(
                        src.at[0, h, pl.ds(Sk - W + st, KV_ROWS), :],
                        dst.at[h, pl.ds(st, KV_ROWS), :],
                        sem_kv.at[which, h]).start(priority=j % 2)

            def wo_pair(j):
                for p in range(2):
                    r = pl.multiple_of((2 * j + p) * wrows, wrows)
                    pltpu.make_async_copy(wo_hbm.at[pl.ds(r, wrows), :], wobuf.at[pl.ds(r, wrows), :],
                                          sem_wo.at[j // wo_pairs_per_group]).start(priority=p)

            def mlp_round(r):
                for s_ in range(4):
                    c = s_ * MS_PER + r
                    def go(c=c):
                        row = pl.multiple_of(c * wrows, wrows)
                        pltpu.make_async_copy(w3t_hbm.at[pl.ds(row, wrows), :], w3buf.at[pl.ds(row, wrows), :],
                                              sem_w.at[0]).start(priority=0)
                        pltpu.make_async_copy(w4_hbm.at[pl.ds(row, wrows), :], w4buf.at[pl.ds(row, wrows), :],
                                              sem_w.at[1]).start(priority=1)
                    if (s_ + 1) * MS_PER <= n_mlp:
                        go()
                    else:
                        pl.when(c < n_mlp)(go)

            def wq_round(i):
                col = pl.multiple_of((i % 2) * wq_cols, wq_cols)
                for s_ in range(8):
                    r = pl.multiple_of((s_ * (n_wq // 8) + i // 2) * wq_rows, wq_rows)
                    pltpu.make_async_copy(
                        wq_hbm.at[pl.ds(r, wq_rows), pl.ds(col, wq_cols)],
                        wqbuf.at[pl.ds(r, wq_rows), pl.ds(col, wq_cols)],
                        sem_w.at[2]).start(priority=s_ % 2)

            with sc("p_issue0"):
                pltpu.make_async_copy(x_hbm, xbuf, sem_x.at[0]).start()
                loop(0, MS_PER, mlp_round)
            with sc("p_ln"):
                pltpu.make_async_copy(x_hbm, xbuf, sem_x.at[0]).wait()
                x = xbuf[0].astype(f32)
                xn = _layernorm(x)
                x1n = _layernorm(xn)
            with sc("p_issue1"):
                loop(0, 2 * n_wq // 8, wq_round)
            with sc("p_mlp"):
                wait_all(w3buf, sem_w.at[0])
                wait_all(w4buf, sem_w.at[1])
                if skip_compute:
                    g_ = x1n
                else:
                    hh = lax.dot_general(x1n.astype(bf16), w3buf[...], (((1,), (1,)), ((), ())),
                                         preferred_element_type=f32)
                    hh = jax.nn.gelu(hh, approximate=True)
                    h2 = jnp.dot(hh.astype(bf16), w4buf[...], preferred_element_type=f32)
                    g_ = jax.nn.silu(xn + h2)
            with sc("p_issue2"):
                loop(0, K0_SPLIT, lambda r: kv_round(0, 0, r))
            with sc("p_q"):
                wait_all(wqbuf, sem_w.at[2])
                if not skip_compute:
                    q = jnp.dot(xn.astype(bf16), wqbuf[...], preferred_element_type=f32).astype(bf16)
                    for h in range(H):
                        q_scr[h] = q[:, h * Dh:(h + 1) * Dh]
            with sc("p_issue4"):
                loop(K0_SPLIT, nblk, lambda r: kv_round(0, 0, r))
                loop(0, AR, lambda r: kv_round(1, 0, r))

            NT = G - AR // RPT
            base = ppr * AR

            def group(g, carry):
                def ktask(j, c):
                    h = g * G + j
                    with sc("k_issue"):
                        @pl.when(j < NT)
                        def _():
                            loop(AR + RPT * j, AR + RPT * (j + 1), lambda r: kv_round(1, g, r))

                        @pl.when(jnp.logical_and(j >= NT, g < NG - 1))
                        def _():
                            loop(RPT * (j - NT), RPT * (j - NT + 1), lambda r: kv_round(0, g + 1, r))

                        @pl.when(jnp.logical_and(j >= NT, g == NG - 1))
                        def _():
                            loop(ppr * RPT * (j - NT), ppr * RPT * (j - NT + 1), wo_pair)
                    with sc("k_wait"):
                        wait_all(kbuf.at[h], sem_kv.at[0, h])
                    with sc("k_task"):
                        if not skip_compute:
                            s = lax.dot_general(q_scr[h], kbuf[h], (((1,), (1,)), ((), ())),
                                                preferred_element_type=f32) * scale
                            m = jnp.max(s, axis=-1, keepdims=True)
                            p = jnp.exp(s - m)
                            l_scr[j] = jnp.broadcast_to(jnp.sum(p, axis=-1, keepdims=True), (1, Dh))
                            p_scr[j] = p.astype(bf16)
                    return c

                lax.fori_loop(0, G, ktask, 0)

                def vtask(j, c):
                    h = g * G + j
                    with sc("v_issue"):
                        @pl.when(jnp.logical_and(j < NT, g < NG - 1))
                        def _():
                            loop(AR + RPT * j, AR + RPT * (j + 1), lambda r: kv_round(0, g + 1, r))

                        @pl.when(jnp.logical_and(j >= NT, g < NG - 1))
                        def _():
                            loop(RPT * (j - NT), RPT * (j - NT + 1), lambda r: kv_round(1, g + 1, r))

                        lo = jnp.where(j == 0, base, jnp.where(j == T1[0], base + T0, 0))
                        hi = jnp.where(j == 0, base + T0, jnp.where(j == T1[0], base + T0 + T1[1], 0))
                        @pl.when(g == NG - 1)
                        def _():
                            loop(lo, hi, wo_pair)
                    with sc("v_wait"):
                        wait_all(vbuf.at[h], sem_kv.at[1, h])
                    with sc("v_task"):
                        if not skip_compute:
                            o = jnp.dot(p_scr[j], vbuf[h], preferred_element_type=f32)
                            o_scr[h] = (o / l_scr[j]).astype(bf16)
                    return c

                lax.fori_loop(0, G, vtask, 0)
                return carry

            lax.fori_loop(0, NG, group, 0)

            with sc("t_issue"):
                loop(base + T0 + T1[1], n_wo, wo_pair)

            def wo_body(gi, acc):
                r0 = pl.multiple_of(gi * (WO_HEADS * Dh), WO_HEADS * Dh)
                wg = wobuf.at[pl.ds(r0, WO_HEADS * Dh), :]
                wait_all(wg, sem_wo.at[gi])
                if skip_compute:
                    return acc
                if WO_HEADS == 1:
                    og = o_scr[gi]
                else:
                    og = jnp.concatenate([o_scr[gi * WO_HEADS + t] for t in range(WO_HEADS)], axis=1)
                return acc + jnp.dot(og, wg[...], preferred_element_type=f32)

            with sc("t_wo"):
                acc = lax.fori_loop(0, n_wo_groups, wo_body, jnp.zeros((1, D), f32))
            with sc("t_final"):
                o_ref[0] = (x + acc * g_).astype(o_ref.dtype)

        return pl.pallas_call(
            kernel,
            in_specs=[pl.BlockSpec(memory_space=pl.ANY)] * 7,
            out_specs=pl.BlockSpec(memory_space=pltpu.VMEM),
            out_shape=jax.ShapeDtypeStruct((B, Sq, D), A_x.dtype),
            scratch_shapes=[
                pltpu.VMEM((1, 1, D), bf16),
                pltpu.VMEM((H, W, Dh), bf16),
                pltpu.VMEM((H, W, Dh), bf16),
                pltpu.VMEM((D, HD), bf16),
                pltpu.VMEM((HD, D), bf16),
                pltpu.VMEM((F, D), bf16),
                pltpu.VMEM((F, D), bf16),
                pltpu.VMEM((H, 1, Dh), bf16),
                pltpu.VMEM((G, 1, W), bf16),
                pltpu.VMEM((G, 1, Dh), f32),
                pltpu.VMEM((H, 1, Dh), bf16),
                pltpu.SemaphoreType.DMA((2,)),
                pltpu.SemaphoreType.DMA((3,)),
                pltpu.SemaphoreType.DMA((2, H)),
                pltpu.SemaphoreType.DMA((n_wo_groups,)),
            ],
            compiler_params=pltpu.CompilerParams(vmem_limit_bytes=100 * 1024 * 1024,
                                                 disable_bounds_checks=True,
                                                 disable_semaphore_checks=True),
        )(A_x, A_k_cache, A_v_cache, A_wq, A_wo, B_w3.T, B_w4)
    return fn


_fn = build(**dict(T0=8))

@jax.jit
def pallas_recurrent_scan__sliding_block_cached__mixer_s_mlp__decode_kernel(A_x, A_k_cache, A_v_cache, A_wq, A_wo, B_x, B_w1, B_w2, B_w3, B_w4):
    return _fn(A_x, A_k_cache, A_v_cache, A_wq, A_wo, B_x, B_w1, B_w2, B_w3, B_w4)
```

```python
import jax
import jax.numpy as jnp
from jax import lax
import jax.experimental.pallas as pl
import jax.experimental.pallas.tpu as pltpu

_EPS = 1e-5
_G = 8
_KV_ROWS = 128
_AHEAD = 8
_K0_SPLIT = 16
_TAIL = ((0, 3), (3, 3))


def _layernorm(x):
    m = jnp.mean(x, axis=-1, keepdims=True)
    d = x - m
    v = jnp.mean(d * d, axis=-1, keepdims=True)
    return d / jnp.sqrt(v + _EPS)


@jax.jit
def pallas_recurrent_scan__sliding_block_cached__mixer_s_mlp__decode_kernel(
    A_x: jax.Array,
    A_k_cache: jax.Array,
    A_v_cache: jax.Array,
    A_wq: jax.Array,
    A_wo: jax.Array,
    B_x: jax.Array,
    B_w1: jax.Array,
    B_w2: jax.Array,
    B_w3: jax.Array,
    B_w4: jax.Array,
):
    B, Sq, D = A_x.shape
    _, H, Sk, Dh = A_k_cache.shape
    W = min(4096, max(256, Sk // 4))
    F = B_w3.shape[1]
    HD = H * Dh
    scale = Dh ** -0.5
    bf16 = jnp.bfloat16
    f32 = jnp.float32
    G = _G

    chunk_bytes = _KV_ROWS * Dh * 2
    n_groups = H // G
    n_blk = W // _KV_ROWS
    per_task = n_blk // G
    n_same = G - _AHEAD // per_task
    w_rows = chunk_bytes // (D * 2)
    n_mlp = F // w_rows
    mlp_per = -(-n_mlp // 4)
    wq_cols = HD // 2
    wq_rows = chunk_bytes // (wq_cols * 2)
    wq_per = D // wq_rows // G
    n_q = Dh // w_rows
    n_wo = HD // (G * w_rows)
    last = n_wo - 1
    assert B == 1 and Sq == 1 and H % G == 0 and H & (H - 1) == 0
    assert W % _KV_ROWS == 0 and n_blk % G == 0 and _AHEAD % per_task == 0
    assert F % w_rows == 0 and wq_rows % 8 == 0 and D % (wq_rows * G) == 0
    assert G == 2 * n_q and n_wo % 2 == 0 and G * w_rows == 2 * Dh
    tail_issued = _AHEAD + sum(n for _, n in _TAIL)
    assert tail_issued <= n_wo

    def kernel(x_hbm, k_hbm, v_hbm, wq_hbm, wo_hbm, w3t_hbm, w4_hbm, o_ref,
               xbuf, kbuf, vbuf, wqbuf, wobuf, w3buf, w4buf,
               q_scr, p_scr, l_scr, o_scr, obc,
               sem_x, sem_w, sem_kv, sem_wo):

        def wait_all(buf, sem):
            pltpu.make_async_copy(buf, buf, sem).wait()

        def loop(lo, hi, f):
            def body(i, c):
                f(i)
                return c
            lax.fori_loop(lo, hi, body, 0)

        def mlp_round(r):
            for s in range(4):
                c = s * mlp_per + r

                def go(c=c):
                    row = pl.multiple_of(c * w_rows, w_rows)
                    pltpu.make_async_copy(w3t_hbm.at[pl.ds(row, w_rows), :],
                                          w3buf.at[pl.ds(row, w_rows), :],
                                          sem_w.at[0]).start(priority=0)
                    pltpu.make_async_copy(w4_hbm.at[pl.ds(row, w_rows), :],
                                          w4buf.at[pl.ds(row, w_rows), :],
                                          sem_w.at[1]).start(priority=1)

                if (s + 1) * mlp_per <= n_mlp:
                    go()
                else:
                    pl.when(c < n_mlp)(go)

        def wq_round(i):
            col = pl.multiple_of((i % 2) * wq_cols, wq_cols)
            for s in range(G):
                row = pl.multiple_of((s * wq_per + i // 2) * wq_rows, wq_rows)
                pltpu.make_async_copy(
                    wq_hbm.at[pl.ds(row, wq_rows), pl.ds(col, wq_cols)],
                    wqbuf.at[pl.ds(row, wq_rows), pl.ds(col, wq_cols)],
                    sem_w.at[2]).start(priority=s % 2)

        def kv_round(which, g, blk):
            src = (k_hbm, v_hbm)[which]
            dst = (kbuf, vbuf)[which]
            st = pl.multiple_of(blk * _KV_ROWS, _KV_ROWS)
            for j in range(G):
                h = g * G + j
                pltpu.make_async_copy(
                    src.at[0, h, pl.ds(Sk - W + st, _KV_ROWS), :],
                    dst.at[h, pl.ds(st, _KV_ROWS), :],
                    sem_kv.at[which, h]).start(priority=j % 2)

        def wo_head(r, b, t):
            return (r + (H // G) * b + (H // 2) * t) & (H - 1)

        def wo_round(r):
            for b in range(n_q):
                for t in range(2):
                    row = pl.multiple_of(wo_head(r, b, t) * Dh + b * w_rows, w_rows)
                    si = r if t == 0 else jnp.where(r == last, n_wo, r)
                    pltpu.make_async_copy(
                        wo_hbm.at[pl.ds(row, w_rows), :],
                        wobuf.at[r, pl.ds((b + n_q * t) * w_rows, w_rows), :],
                        sem_wo.at[si]).start(priority=t)

        x_copy = pltpu.make_async_copy(x_hbm, xbuf, sem_x.at[0])
        x_copy.start()
        loop(0, mlp_per, mlp_round)
        x_copy.wait()
        x = xbuf[0].astype(f32)
        xn = _layernorm(x)
        x1n = _layernorm(xn)

        loop(0, 2 * wq_per, wq_round)
        wait_all(w3buf, sem_w.at[0])
        wait_all(w4buf, sem_w.at[1])
        hh = lax.dot_general(x1n.astype(bf16), w3buf[...], (((1,), (1,)), ((), ())),
                             preferred_element_type=f32)
        hh = jax.nn.gelu(hh, approximate=True)
        h2 = jnp.dot(hh.astype(bf16), w4buf[...], preferred_element_type=f32)
        gate = jax.nn.silu(xn + h2)

        loop(0, _K0_SPLIT, lambda r: kv_round(0, 0, r))
        wait_all(wqbuf, sem_w.at[2])
        q = jnp.dot(xn.astype(bf16), wqbuf[...], preferred_element_type=f32).astype(bf16)
        for h in range(H):
            q_scr[h] = q[:, h * Dh:(h + 1) * Dh]
        loop(_K0_SPLIT, n_blk, lambda r: kv_round(0, 0, r))
        loop(0, _AHEAD, lambda r: kv_round(1, 0, r))

        def group(g, carry):
            more = g < n_groups - 1

            def score_task(j, c):
                h = g * G + j

                @pl.when(j < n_same)
                def _():
                    lo = _AHEAD + per_task * j
                    loop(lo, lo + per_task, lambda r: kv_round(1, g, r))

                @pl.when(jnp.logical_and(j >= n_same, more))
                def _():
                    lo = per_task * (j - n_same)
                    loop(lo, lo + per_task, lambda r: kv_round(0, g + 1, r))

                @pl.when(jnp.logical_and(j >= n_same, jnp.logical_not(more)))
                def _():
                    lo = per_task * (j - n_same)
                    loop(lo, lo + per_task, wo_round)

                wait_all(kbuf.at[h], sem_kv.at[0, h])
                s = lax.dot_general(q_scr[h], kbuf[h], (((1,), (1,)), ((), ())),
                                    preferred_element_type=f32) * scale
                m = jnp.max(s, axis=-1, keepdims=True)
                p = jnp.exp(s - m)
                l_scr[j] = jnp.broadcast_to(jnp.sum(p, axis=-1, keepdims=True), (1, Dh))
                p_scr[j] = p.astype(bf16)
                return c

            lax.fori_loop(0, G, score_task, 0)

            def value_task(j, c):
                h = g * G + j

                @pl.when(jnp.logical_and(j < n_same, more))
                def _():
                    lo = _AHEAD + per_task * j
                    loop(lo, lo + per_task, lambda r: kv_round(0, g + 1, r))

                @pl.when(jnp.logical_and(j >= n_same, more))
                def _():
                    lo = per_task * (j - n_same)
                    loop(lo, lo + per_task, lambda r: kv_round(1, g + 1, r))

                @pl.when(jnp.logical_not(more))
                def _():
                    lo, hi, at = 0, 0, _AHEAD
                    for task, n in _TAIL:
                        lo = jnp.where(j == task, at, lo)
                        hi = jnp.where(j == task, at + n, hi)
                        at += n
                    loop(lo, hi, wo_round)

                wait_all(vbuf.at[h], sem_kv.at[1, h])
                o = jnp.dot(p_scr[j], vbuf[h], preferred_element_type=f32)
                o_scr[h] = o / l_scr[j]
                return c

            lax.fori_loop(0, G, value_task, 0)
            return carry

        lax.fori_loop(0, n_groups, group, 0)
        loop(tail_issued, n_wo, wo_round)

        def wo_lhs(r):
            lane_q = lax.broadcasted_iota(jnp.int32, (1, Dh), 1) // w_rows
            halves = []
            for t in range(2):
                v = o_scr[wo_head(r, 0, t)]
                for b in range(1, n_q):
                    v = jnp.where(lane_q == b, o_scr[wo_head(r, b, t)], v)
                halves.append(v)
            return jnp.concatenate(halves, axis=1).astype(bf16)

        lhs_last = wo_lhs(last)
        obc[...] = jnp.broadcast_to(lhs_last[:, Dh:].astype(f32), (Dh, Dh)).T

        def wo_two_rounds(i, acc):
            for u in range(2):
                wait_all(wobuf.at[2 * i + u], sem_wo.at[2 * i + u])
            for u in range(2):
                r = 2 * i + u
                acc = acc + jnp.dot(wo_lhs(r), wobuf[r], preferred_element_type=f32)
            return acc

        acc = lax.fori_loop(0, n_wo // 2 - 1, wo_two_rounds, jnp.zeros((1, D), f32))

        wa = wobuf.at[last, pl.ds(0, Dh), :]
        wb = wobuf.at[last, pl.ds(Dh, Dh), :]
        lhs_prev = wo_lhs(last - 1)
        wait_all(wobuf.at[last - 1], sem_wo.at[last - 1])
        wait_all(wa, sem_wo.at[last])
        acc = acc + jnp.dot(lhs_prev, wobuf[last - 1], preferred_element_type=f32)
        acc = acc + jnp.dot(lhs_last[:, :Dh], wa[...], preferred_element_type=f32)
        wait_all(wb, sem_wo.at[n_wo])
        prod = wb[...].astype(f32) * jnp.concatenate([obc[...]] * (D // Dh), axis=1)
        acc = acc + jnp.sum(prod, axis=0, keepdims=True)

        o_ref[0] = (x + acc * gate).astype(o_ref.dtype)

    return pl.pallas_call(
        kernel,
        in_specs=[pl.BlockSpec(memory_space=pl.ANY)] * 7,
        out_specs=pl.BlockSpec(memory_space=pltpu.VMEM),
        out_shape=jax.ShapeDtypeStruct((B, Sq, D), A_x.dtype),
        scratch_shapes=[
            pltpu.VMEM((1, 1, D), bf16),
            pltpu.VMEM((H, W, Dh), bf16),
            pltpu.VMEM((H, W, Dh), bf16),
            pltpu.VMEM((D, HD), bf16),
            pltpu.VMEM((n_wo, G * w_rows, D), bf16),
            pltpu.VMEM((F, D), bf16),
            pltpu.VMEM((F, D), bf16),
            pltpu.VMEM((H, 1, Dh), bf16),
            pltpu.VMEM((G, 1, W), bf16),
            pltpu.VMEM((G, 1, Dh), f32),
            pltpu.VMEM((H, 1, Dh), f32),
            pltpu.VMEM((Dh, Dh), f32),
            pltpu.SemaphoreType.DMA((1,)),
            pltpu.SemaphoreType.DMA((3,)),
            pltpu.SemaphoreType.DMA((2, H)),
            pltpu.SemaphoreType.DMA((n_wo + 1,)),
        ],
        compiler_params=pltpu.CompilerParams(
            vmem_limit_bytes=100 * 1024 * 1024,
            disable_bounds_checks=True,
            disable_semaphore_checks=True,
        ),
    )(A_x, A_k_cache, A_v_cache, A_wq, A_wo, B_w3.T, B_w4)
```

```python
import jax
import jax.numpy as jnp
from jax import lax
import jax.experimental.pallas as pl
import jax.experimental.pallas.tpu as pltpu

_EPS = 1e-5
_G = 8
_KV_ROWS = 128
_KV_SHIFT = 16
_AHEAD = 8
_K0_SPLIT = 16
_TAIL = ((0, 3), (3, 3))


def _layernorm(x):
    m = jnp.mean(x, axis=-1, keepdims=True)
    d = x - m
    v = jnp.mean(d * d, axis=-1, keepdims=True)
    return d / jnp.sqrt(v + _EPS)


@jax.jit
def pallas_recurrent_scan__sliding_block_cached__mixer_s_mlp__decode_kernel(
    A_x: jax.Array,
    A_k_cache: jax.Array,
    A_v_cache: jax.Array,
    A_wq: jax.Array,
    A_wo: jax.Array,
    B_x: jax.Array,
    B_w1: jax.Array,
    B_w2: jax.Array,
    B_w3: jax.Array,
    B_w4: jax.Array,
):
    B, Sq, D = A_x.shape
    _, H, Sk, Dh = A_k_cache.shape
    W = min(4096, max(256, Sk // 4))
    F = B_w3.shape[1]
    HD = H * Dh
    scale = Dh ** -0.5
    bf16 = jnp.bfloat16
    f32 = jnp.float32
    G = _G

    chunk_bytes = _KV_ROWS * Dh * 2
    n_groups = H // G
    n_blk = W // _KV_ROWS
    per_task = n_blk // G
    n_same = G - _AHEAD // per_task
    w_rows = chunk_bytes // (D * 2)
    n_mlp = F // w_rows
    mlp_per = -(-n_mlp // 4)
    wq_cols = HD // 2
    wq_rows = chunk_bytes // (wq_cols * 2)
    wq_per = D // wq_rows // G
    n_q = Dh // w_rows
    n_wo = HD // (G * w_rows)
    last = n_wo - 1
    assert B == 1 and Sq == 1 and H % G == 0 and H & (H - 1) == 0
    assert W % _KV_ROWS == 0 and n_blk % G == 0 and _AHEAD % per_task == 0
    assert F % w_rows == 0 and wq_rows % 8 == 0 and D % (wq_rows * G) == 0
    assert G == 2 * n_q and n_wo % 2 == 0 and G * w_rows == 2 * Dh
    tail_issued = _AHEAD + sum(n for _, n in _TAIL)
    assert tail_issued <= n_wo

    def kernel(x_hbm, k_hbm, v_hbm, wq_hbm, wo_hbm, w3t_hbm, w4_hbm, o_ref,
               xbuf, kbuf, vbuf, wqbuf, wobuf, w3buf, w4buf,
               q_scr, p_scr, l_scr, o_scr, obc,
               sem_x, sem_w, sem_kv, sem_wo):

        def wait_all(buf, sem):
            pltpu.make_async_copy(buf, buf, sem).wait()

        def loop(lo, hi, f):
            def body(i, c):
                f(i)
                return c
            lax.fori_loop(lo, hi, body, 0)

        def mlp_round(r):
            for s in range(4):
                c = s * mlp_per + r

                def go(c=c):
                    row = pl.multiple_of(c * w_rows, w_rows)
                    pltpu.make_async_copy(w3t_hbm.at[pl.ds(row, w_rows), :],
                                          w3buf.at[pl.ds(row, w_rows), :],
                                          sem_w.at[0]).start(priority=0)
                    pltpu.make_async_copy(w4_hbm.at[pl.ds(row, w_rows), :],
                                          w4buf.at[pl.ds(row, w_rows), :],
                                          sem_w.at[1]).start(priority=1)

                if (s + 1) * mlp_per <= n_mlp:
                    go()
                else:
                    pl.when(c < n_mlp)(go)

        def wq_round(i):
            col = pl.multiple_of((i % 2) * wq_cols, wq_cols)
            for s in range(G):
                row = pl.multiple_of((s * wq_per + i // 2) * wq_rows, wq_rows)
                pltpu.make_async_copy(
                    wq_hbm.at[pl.ds(row, wq_rows), pl.ds(col, wq_cols)],
                    wqbuf.at[pl.ds(row, wq_rows), pl.ds(col, wq_cols)],
                    sem_w.at[2]).start(priority=s % 2)

        def kv_round(which, g, blk):
            src = (k_hbm, v_hbm)[which]
            dst = (kbuf, vbuf)[which]

            def chunks(st, rows):
                for j in range(G):
                    h = g * G + j
                    pltpu.make_async_copy(
                        src.at[0, h, pl.ds(Sk - W + st, rows), :],
                        dst.at[h, pl.ds(st, rows), :],
                        sem_kv.at[which, h]).start(priority=j % 2)

            @pl.when(blk == 0)
            def _():
                chunks(0, _KV_ROWS - _KV_SHIFT)

            @pl.when(jnp.logical_and(blk > 0, blk < n_blk - 1))
            def _():
                chunks(pl.multiple_of(blk * _KV_ROWS - _KV_SHIFT, 8), _KV_ROWS)

            @pl.when(blk == n_blk - 1)
            def _():
                chunks((n_blk - 1) * _KV_ROWS - _KV_SHIFT, _KV_ROWS + _KV_SHIFT)

        def wo_head(r, b, t):
            return (r + (H // G) * b + (H // 2) * t) & (H - 1)

        def wo_round(r):
            for b in range(n_q):
                for t in range(2):
                    row = pl.multiple_of(wo_head(r, b, t) * Dh + b * w_rows, w_rows)
                    si = r if t == 0 else jnp.where(r == last, n_wo, r)
                    pltpu.make_async_copy(
                        wo_hbm.at[pl.ds(row, w_rows), :],
                        wobuf.at[r, pl.ds((b + n_q * t) * w_rows, w_rows), :],
                        sem_wo.at[si]).start(priority=t)

        x_copy = pltpu.make_async_copy(x_hbm, xbuf, sem_x.at[0])
        x_copy.start()
        loop(0, mlp_per, mlp_round)
        x_copy.wait()
        x = xbuf[0].astype(f32)
        xn = _layernorm(x)
        x1n = _layernorm(xn)

        loop(0, 2 * wq_per, wq_round)
        wait_all(w3buf, sem_w.at[0])
        wait_all(w4buf, sem_w.at[1])
        hh = lax.dot_general(x1n.astype(bf16), w3buf[...], (((1,), (1,)), ((), ())),
                             preferred_element_type=f32)
        hh = jax.nn.gelu(hh, approximate=True)
        h2 = jnp.dot(hh.astype(bf16), w4buf[...], preferred_element_type=f32)
        gate = jax.nn.silu(xn + h2)

        loop(0, _K0_SPLIT, lambda r: kv_round(0, 0, r))
        wait_all(wqbuf, sem_w.at[2])
        q = jnp.dot(xn.astype(bf16), wqbuf[...], preferred_element_type=f32).astype(bf16)
        for h in range(H):
            q_scr[h] = q[:, h * Dh:(h + 1) * Dh]
        loop(_K0_SPLIT, n_blk, lambda r: kv_round(0, 0, r))
        loop(0, _AHEAD, lambda r: kv_round(1, 0, r))

        def group(g, carry):
            more = g < n_groups - 1

            def score_task(j, c):
                h = g * G + j

                @pl.when(j < n_same)
                def _():
                    lo = _AHEAD + per_task * j
                    loop(lo, lo + per_task, lambda r: kv_round(1, g, r))

                @pl.when(jnp.logical_and(j >= n_same, more))
                def _():
                    lo = per_task * (j - n_same)
                    loop(lo, lo + per_task, lambda r: kv_round(0, g + 1, r))

                @pl.when(jnp.logical_and(j >= n_same, jnp.logical_not(more)))
                def _():
                    lo = per_task * (j - n_same)
                    loop(lo, lo + per_task, wo_round)

                wait_all(kbuf.at[h], sem_kv.at[0, h])
                s = lax.dot_general(q_scr[h], kbuf[h], (((1,), (1,)), ((), ())),
                                    preferred_element_type=f32) * scale
                m = jnp.max(s, axis=-1, keepdims=True)
                p = jnp.exp(s - m)
                l_scr[j] = jnp.broadcast_to(jnp.sum(p, axis=-1, keepdims=True), (1, Dh))
                p_scr[j] = p.astype(bf16)
                return c

            lax.fori_loop(0, G, score_task, 0)

            def value_task(j, c):
                h = g * G + j

                @pl.when(jnp.logical_and(j < n_same, more))
                def _():
                    lo = _AHEAD + per_task * j
                    loop(lo, lo + per_task, lambda r: kv_round(0, g + 1, r))

                @pl.when(jnp.logical_and(j >= n_same, more))
                def _():
                    lo = per_task * (j - n_same)
                    loop(lo, lo + per_task, lambda r: kv_round(1, g + 1, r))

                @pl.when(jnp.logical_not(more))
                def _():
                    lo, hi, at = 0, 0, _AHEAD
                    for task, n in _TAIL:
                        lo = jnp.where(j == task, at, lo)
                        hi = jnp.where(j == task, at + n, hi)
                        at += n
                    loop(lo, hi, wo_round)

                wait_all(vbuf.at[h], sem_kv.at[1, h])
                o = jnp.dot(p_scr[j], vbuf[h], preferred_element_type=f32)
                o_scr[h] = o / l_scr[j]
                return c

            lax.fori_loop(0, G, value_task, 0)
            return carry

        lax.fori_loop(0, n_groups, group, 0)
        loop(tail_issued, n_wo, wo_round)

        def wo_lhs(r):
            lane_q = lax.broadcasted_iota(jnp.int32, (1, Dh), 1) // w_rows
            halves = []
            for t in range(2):
                v = o_scr[wo_head(r, 0, t)]
                for b in range(1, n_q):
                    v = jnp.where(lane_q == b, o_scr[wo_head(r, b, t)], v)
                halves.append(v)
            return jnp.concatenate(halves, axis=1).astype(bf16)

        lhs_last = wo_lhs(last)
        obc[...] = jnp.broadcast_to(lhs_last[:, Dh:].astype(f32), (Dh, Dh)).T

        def wo_two_rounds(i, acc):
            for u in range(2):
                wait_all(wobuf.at[2 * i + u], sem_wo.at[2 * i + u])
            for u in range(2):
                r = 2 * i + u
                acc = acc + jnp.dot(wo_lhs(r), wobuf[r], preferred_element_type=f32)
            return acc

        acc = lax.fori_loop(0, n_wo // 2 - 1, wo_two_rounds, jnp.zeros((1, D), f32))

        wa = wobuf.at[last, pl.ds(0, Dh), :]
        wb = wobuf.at[last, pl.ds(Dh, Dh), :]
        lhs_prev = wo_lhs(last - 1)
        wait_all(wobuf.at[last - 1], sem_wo.at[last - 1])
        wait_all(wa, sem_wo.at[last])
        acc = acc + jnp.dot(lhs_prev, wobuf[last - 1], preferred_element_type=f32)
        acc = acc + jnp.dot(lhs_last[:, :Dh], wa[...], preferred_element_type=f32)
        wait_all(wb, sem_wo.at[n_wo])
        prod = wb[...].astype(f32) * jnp.concatenate([obc[...]] * (D // Dh), axis=1)
        acc = acc + jnp.sum(prod, axis=0, keepdims=True)

        o_ref[0] = (x + acc * gate).astype(o_ref.dtype)

    return pl.pallas_call(
        kernel,
        in_specs=[pl.BlockSpec(memory_space=pl.ANY)] * 7,
        out_specs=pl.BlockSpec(memory_space=pltpu.VMEM),
        out_shape=jax.ShapeDtypeStruct((B, Sq, D), A_x.dtype),
        scratch_shapes=[
            pltpu.VMEM((1, 1, D), bf16),
            pltpu.VMEM((H, W, Dh), bf16),
            pltpu.VMEM((H, W, Dh), bf16),
            pltpu.VMEM((D, HD), bf16),
            pltpu.VMEM((n_wo, G * w_rows, D), bf16),
            pltpu.VMEM((F, D), bf16),
            pltpu.VMEM((F, D), bf16),
            pltpu.VMEM((H, 1, Dh), bf16),
            pltpu.VMEM((G, 1, W), bf16),
            pltpu.VMEM((G, 1, Dh), f32),
            pltpu.VMEM((H, 1, Dh), f32),
            pltpu.VMEM((Dh, Dh), f32),
            pltpu.SemaphoreType.DMA((1,)),
            pltpu.SemaphoreType.DMA((3,)),
            pltpu.SemaphoreType.DMA((2, H)),
            pltpu.SemaphoreType.DMA((n_wo + 1,)),
        ],
        compiler_params=pltpu.CompilerParams(
            vmem_limit_bytes=100 * 1024 * 1024,
            disable_bounds_checks=True,
            disable_semaphore_checks=True,
        ),
    )(A_x, A_k_cache, A_v_cache, A_wq, A_wo, B_w3.T, B_w4)
```

```python
import jax
import jax.numpy as jnp
from jax import lax
import jax.experimental.pallas as pl
import jax.experimental.pallas.tpu as pltpu

_EPS = 1e-5
_G = 8
_KV_ROWS = 128
_KV_SHIFT = 16
_WARM_ROUNDS = 4
_AHEAD = 8
_K0_SPLIT = 16
_TAIL = ((0, 3), (3, 3))


def _layernorm(x):
    m = jnp.mean(x, axis=-1, keepdims=True)
    d = x - m
    v = jnp.mean(d * d, axis=-1, keepdims=True)
    return d / jnp.sqrt(v + _EPS)


@jax.jit
def pallas_recurrent_scan__sliding_block_cached__mixer_s_mlp__decode_kernel(
    A_x: jax.Array,
    A_k_cache: jax.Array,
    A_v_cache: jax.Array,
    A_wq: jax.Array,
    A_wo: jax.Array,
    B_x: jax.Array,
    B_w1: jax.Array,
    B_w2: jax.Array,
    B_w3: jax.Array,
    B_w4: jax.Array,
):
    B, Sq, D = A_x.shape
    _, H, Sk, Dh = A_k_cache.shape
    W = min(4096, max(256, Sk // 4))
    F = B_w3.shape[1]
    HD = H * Dh
    scale = Dh ** -0.5
    bf16 = jnp.bfloat16
    f32 = jnp.float32
    G = _G

    chunk_bytes = _KV_ROWS * Dh * 2
    n_groups = H // G
    n_blk = W // _KV_ROWS
    per_task = n_blk // G
    n_same = G - _AHEAD // per_task
    w_rows = chunk_bytes // (D * 2)
    n_mlp = F // w_rows
    mlp_per = -(-n_mlp // 4)
    wq_cols = HD // 2
    wq_rows = chunk_bytes // (wq_cols * 2)
    wq_per = D // wq_rows // G
    n_q = Dh // w_rows
    n_wo = HD // (G * w_rows)
    last = n_wo - 1
    assert B == 1 and Sq == 1 and H % G == 0 and H & (H - 1) == 0
    assert W % _KV_ROWS == 0 and n_blk % G == 0 and _AHEAD % per_task == 0
    assert F % w_rows == 0 and wq_rows % 8 == 0 and D % (wq_rows * G) == 0
    assert G == 2 * n_q and n_wo % 2 == 0 and G * w_rows == 2 * Dh
    tail_issued = _AHEAD + sum(n for _, n in _TAIL)
    assert tail_issued <= n_wo

    def kernel(x_hbm, k_hbm, v_hbm, wq_hbm, wo_hbm, w3t_hbm, w4_hbm, o_ref,
               xbuf, kbuf, vbuf, wqbuf, wobuf, w3buf, w4buf,
               q_scr, p_scr, l_scr, o_scr, obc,
               sem_x, sem_w, sem_kv, sem_wo):

        def wait_all(buf, sem):
            pltpu.make_async_copy(buf, buf, sem).wait()

        def loop(lo, hi, f):
            def body(i, c):
                f(i)
                return c
            lax.fori_loop(lo, hi, body, 0)

        def mlp_round(r, w3_priority=0):
            for s in range(4):
                c = s * mlp_per + r

                def go(c=c):
                    row = pl.multiple_of(c * w_rows, w_rows)
                    pltpu.make_async_copy(w3t_hbm.at[pl.ds(row, w_rows), :],
                                          w3buf.at[pl.ds(row, w_rows), :],
                                          sem_w.at[0]).start(priority=w3_priority)
                    pltpu.make_async_copy(w4_hbm.at[pl.ds(row, w_rows), :],
                                          w4buf.at[pl.ds(row, w_rows), :],
                                          sem_w.at[1]).start(priority=1)

                if (s + 1) * mlp_per <= n_mlp:
                    go()
                else:
                    pl.when(c < n_mlp)(go)

        def wq_round(i):
            col = pl.multiple_of((i % 2) * wq_cols, wq_cols)
            for s in range(G):
                row = pl.multiple_of((s * wq_per + i // 2) * wq_rows, wq_rows)
                pltpu.make_async_copy(
                    wq_hbm.at[pl.ds(row, wq_rows), pl.ds(col, wq_cols)],
                    wqbuf.at[pl.ds(row, wq_rows), pl.ds(col, wq_cols)],
                    sem_w.at[2]).start(priority=s % 2)

        def kv_round(which, g, blk):
            src = (k_hbm, v_hbm)[which]
            dst = (kbuf, vbuf)[which]

            def chunks(st, rows):
                for j in range(G):
                    h = g * G + j
                    pltpu.make_async_copy(
                        src.at[0, h, pl.ds(Sk - W + st, rows), :],
                        dst.at[h, pl.ds(st, rows), :],
                        sem_kv.at[which, h]).start(priority=j % 2)

            @pl.when(blk == 0)
            def _():
                chunks(0, _KV_ROWS - _KV_SHIFT)

            @pl.when(jnp.logical_and(blk > 0, blk < n_blk - 1))
            def _():
                chunks(pl.multiple_of(blk * _KV_ROWS - _KV_SHIFT, 8), _KV_ROWS)

            @pl.when(blk == n_blk - 1)
            def _():
                chunks((n_blk - 1) * _KV_ROWS - _KV_SHIFT, _KV_ROWS + _KV_SHIFT)

        def wo_head(r, b, t):
            return (r + (H // G) * b + (H // 2) * t) & (H - 1)

        def wo_round(r):
            for b in range(n_q):
                for t in range(2):
                    row = pl.multiple_of(wo_head(r, b, t) * Dh + b * w_rows, w_rows)
                    si = r if t == 0 else jnp.where(r == last, n_wo, r)
                    pltpu.make_async_copy(
                        wo_hbm.at[pl.ds(row, w_rows), :],
                        wobuf.at[r, pl.ds((b + n_q * t) * w_rows, w_rows), :],
                        sem_wo.at[si]).start(priority=t)

        x_copy = pltpu.make_async_copy(x_hbm, xbuf, sem_x.at[0])
        x_copy.start()
        loop(0, _WARM_ROUNDS, lambda r: mlp_round(r, 1))
        loop(_WARM_ROUNDS, mlp_per, mlp_round)
        x_copy.wait()
        x = xbuf[0].astype(f32)
        xn = _layernorm(x)
        x1n = _layernorm(xn)

        loop(0, 2 * wq_per, wq_round)
        wait_all(w3buf, sem_w.at[0])
        wait_all(w4buf, sem_w.at[1])
        hh = lax.dot_general(x1n.astype(bf16), w3buf[...], (((1,), (1,)), ((), ())),
                             preferred_element_type=f32)
        hh = jax.nn.gelu(hh, approximate=True)
        h2 = jnp.dot(hh.astype(bf16), w4buf[...], preferred_element_type=f32)
        gate = jax.nn.silu(xn + h2)

        loop(0, _K0_SPLIT, lambda r: kv_round(0, 0, r))
        wait_all(wqbuf, sem_w.at[2])
        q = jnp.dot(xn.astype(bf16), wqbuf[...], preferred_element_type=f32).astype(bf16)
        for h in range(H):
            q_scr[h] = q[:, h * Dh:(h + 1) * Dh]
        loop(_K0_SPLIT, n_blk, lambda r: kv_round(0, 0, r))
        loop(0, _AHEAD, lambda r: kv_round(1, 0, r))

        def group(g, carry):
            more = g < n_groups - 1

            def score_task(j, c):
                h = g * G + j

                @pl.when(j < n_same)
                def _():
                    lo = _AHEAD + per_task * j
                    loop(lo, lo + per_task, lambda r: kv_round(1, g, r))

                @pl.when(jnp.logical_and(j >= n_same, more))
                def _():
                    lo = per_task * (j - n_same)
                    loop(lo, lo + per_task, lambda r: kv_round(0, g + 1, r))

                @pl.when(jnp.logical_and(j >= n_same, jnp.logical_not(more)))
                def _():
                    lo = per_task * (j - n_same)
                    loop(lo, lo + per_task, wo_round)

                wait_all(kbuf.at[h], sem_kv.at[0, h])
                s = lax.dot_general(q_scr[h], kbuf[h], (((1,), (1,)), ((), ())),
                                    preferred_element_type=f32) * scale
                m = jnp.max(s, axis=-1, keepdims=True)
                p = jnp.exp(s - m)
                l_scr[j] = jnp.broadcast_to(jnp.sum(p, axis=-1, keepdims=True), (1, Dh))
                p_scr[j] = p.astype(bf16)
                return c

            lax.fori_loop(0, G, score_task, 0)

            def value_task(j, c):
                h = g * G + j

                @pl.when(jnp.logical_and(j < n_same, more))
                def _():
                    lo = _AHEAD + per_task * j
                    loop(lo, lo + per_task, lambda r: kv_round(0, g + 1, r))

                @pl.when(jnp.logical_and(j >= n_same, more))
                def _():
                    lo = per_task * (j - n_same)
                    loop(lo, lo + per_task, lambda r: kv_round(1, g + 1, r))

                @pl.when(jnp.logical_not(more))
                def _():
                    lo, hi, at = 0, 0, _AHEAD
                    for task, n in _TAIL:
                        lo = jnp.where(j == task, at, lo)
                        hi = jnp.where(j == task, at + n, hi)
                        at += n
                    loop(lo, hi, wo_round)

                wait_all(vbuf.at[h], sem_kv.at[1, h])
                o = jnp.dot(p_scr[j], vbuf[h], preferred_element_type=f32)
                o_scr[h] = o / l_scr[j]
                return c

            lax.fori_loop(0, G, value_task, 0)
            return carry

        lax.fori_loop(0, n_groups, group, 0)
        loop(tail_issued, n_wo, wo_round)

        def wo_lhs(r):
            lane_q = lax.broadcasted_iota(jnp.int32, (1, Dh), 1) // w_rows
            halves = []
            for t in range(2):
                v = o_scr[wo_head(r, 0, t)]
                for b in range(1, n_q):
                    v = jnp.where(lane_q == b, o_scr[wo_head(r, b, t)], v)
                halves.append(v)
            return jnp.concatenate(halves, axis=1).astype(bf16)

        lhs_last = wo_lhs(last)
        obc[...] = jnp.broadcast_to(lhs_last[:, Dh:].astype(f32), (Dh, Dh)).T

        def wo_two_rounds(i, acc):
            for u in range(2):
                wait_all(wobuf.at[2 * i + u], sem_wo.at[2 * i + u])
            for u in range(2):
                r = 2 * i + u
                acc = acc + jnp.dot(wo_lhs(r), wobuf[r], preferred_element_type=f32)
            return acc

        acc = lax.fori_loop(0, n_wo // 2 - 1, wo_two_rounds, jnp.zeros((1, D), f32))

        wa = wobuf.at[last, pl.ds(0, Dh), :]
        wb = wobuf.at[last, pl.ds(Dh, Dh), :]
        lhs_prev = wo_lhs(last - 1)
        wait_all(wobuf.at[last - 1], sem_wo.at[last - 1])
        wait_all(wa, sem_wo.at[last])
        acc = acc + jnp.dot(lhs_prev, wobuf[last - 1], preferred_element_type=f32)
        acc = acc + jnp.dot(lhs_last[:, :Dh], wa[...], preferred_element_type=f32)
        wait_all(wb, sem_wo.at[n_wo])
        prod = wb[...].astype(f32) * jnp.concatenate([obc[...]] * (D // Dh), axis=1)
        acc = acc + jnp.sum(prod, axis=0, keepdims=True)

        o_ref[0] = (x + acc * gate).astype(o_ref.dtype)

    return pl.pallas_call(
        kernel,
        in_specs=[pl.BlockSpec(memory_space=pl.ANY)] * 7,
        out_specs=pl.BlockSpec(memory_space=pltpu.VMEM),
        out_shape=jax.ShapeDtypeStruct((B, Sq, D), A_x.dtype),
        scratch_shapes=[
            pltpu.VMEM((1, 1, D), bf16),
            pltpu.VMEM((H, W, Dh), bf16),
            pltpu.VMEM((H, W, Dh), bf16),
            pltpu.VMEM((D, HD), bf16),
            pltpu.VMEM((n_wo, G * w_rows, D), bf16),
            pltpu.VMEM((F, D), bf16),
            pltpu.VMEM((F, D), bf16),
            pltpu.VMEM((H, 1, Dh), bf16),
            pltpu.VMEM((G, 1, W), bf16),
            pltpu.VMEM((G, 1, Dh), f32),
            pltpu.VMEM((H, 1, Dh), f32),
            pltpu.VMEM((Dh, Dh), f32),
            pltpu.SemaphoreType.DMA((1,)),
            pltpu.SemaphoreType.DMA((3,)),
            pltpu.SemaphoreType.DMA((2, H)),
            pltpu.SemaphoreType.DMA((n_wo + 1,)),
        ],
        compiler_params=pltpu.CompilerParams(
            vmem_limit_bytes=100 * 1024 * 1024,
            disable_bounds_checks=True,
            disable_semaphore_checks=True,
        ),
    )(A_x, A_k_cache, A_v_cache, A_wq, A_wo, B_w3.T, B_w4)
```
